```python
import os as _os
_os.environ.setdefault("JAX_PLATFORMS", "cpu")
import jax
import jax.numpy as jnp

def _softmax(x, axis=-1):
    return jax.nn.softmax(x, axis=axis)
def _gelu(x):
    return jax.nn.gelu(x, approximate=True)
def _silu(x):
    return jax.nn.silu(x)
def _sigmoid(x):
    return jax.nn.sigmoid(x)
def _layernorm(x, axis=-1, eps=1e-5):
    m = jnp.mean(x, axis=axis, keepdims=True)
    v = jnp.var(x, axis=axis, keepdims=True)
    return (x - m) / jnp.sqrt(v + eps)
def _scatter_add(tgt, idx, src, axis=0):
    return tgt.at[idx].add(src)
def _segment_sum(src, seg, n):
    return jax.ops.segment_sum(src, seg, n)
class _Rng:
    def __init__(self, key):
        self._k = key
    def _next(self):
        self._k, sub = jax.random.split(self._k)
        return sub
    def normal(self, shape):
        return jax.random.normal(self._next(), shape, dtype=jnp.bfloat16)
    def randint(self, lo, hi, shape):
        return jax.random.randint(self._next(), shape, lo, hi, dtype=jnp.int32)
    def uniform(self, shape, lo=0.0, hi=1.0):
        return jax.random.uniform(self._next(), shape, jnp.bfloat16, lo, hi)
    def permutation(self, n):
        return jax.random.permutation(self._next(), n)


kernel_name = 'standalone__mha_softmax__near_ridge'

def setup_inputs():
    _rng = _Rng(jax.random.key(int.from_bytes(__import__("os").urandom(4), "little")))
    _w = (lambda a: (lambda t: t.astype(jnp.bfloat16) if jnp.issubdtype(t.dtype, jnp.floating) else t)(jnp.asarray(a)))
    B, H, Sq, Sk, D = 8, 32, 384, 512, 128
    return {
        "q": _w((lambda *s: _rng.normal(s) * 0.4)(B, H, Sq, D)),
        "k": _w((lambda *s: _rng.normal(s) * 0.4)(B, H, Sk, D)),
        "v": _w((lambda *s: _rng.normal(s) * 0.05)(B, H, Sk, D)),
    }

def reference(q, k, v):
    scale = q.shape[-1] ** -0.5
    scores = jnp.einsum("bhqd,bhkd->bhqk", q, k) * scale
    p = _softmax(scores, axis=-1)
    return jnp.einsum("bhqk,bhkd->bhqd", p, v)
```

```python
import functools
import math

import jax
import jax.numpy as jnp
import jax.experimental.pallas as pl
import jax.experimental.pallas.tpu as pltpu


def _attn_kernel(q_ref, k_ref, v_ref, o_ref, *, heads, c):
    for h in range(heads):
        q = q_ref[h]
        k = k_ref[h]
        v = v_ref[h]
        s = jax.lax.dot_general(q, k, (((1,), (1,)), ((), ())),
                                preferred_element_type=jnp.float32)
        m = jnp.max(s, axis=-1, keepdims=True)
        p = jnp.exp2((s - m) * c)
        l = jnp.sum(p, axis=-1, keepdims=True)
        o = jnp.dot(p.astype(jnp.bfloat16), v, preferred_element_type=jnp.float32)
        o_ref[h] = (o * (1.0 / l)).astype(o_ref.dtype)


@jax.jit
def pallas_standalone__mha_softmax__near_ridge_kernel(q, k, v):
    B, H, Sq, D = q.shape
    Sk = k.shape[2]
    BH = B * H
    G = 4
    c = (D ** -0.5) * math.log2(math.e)
    q3 = q.reshape(BH, Sq, D)
    k3 = k.reshape(BH, Sk, D)
    v3 = v.reshape(BH, Sk, D)
    out = pl.pallas_call(
        functools.partial(_attn_kernel, heads=G, c=c),
        grid=(BH // G,),
        in_specs=[
            pl.BlockSpec((G, Sq, D), lambda i: (i, 0, 0)),
            pl.BlockSpec((G, Sk, D), lambda i: (i, 0, 0)),
            pl.BlockSpec((G, Sk, D), lambda i: (i, 0, 0)),
        ],
        out_specs=pl.BlockSpec((G, Sq, D), lambda i: (i, 0, 0)),
        out_shape=jax.ShapeDtypeStruct((BH, Sq, D), q.dtype),
        compiler_params=pltpu.CompilerParams(
            dimension_semantics=("arbitrary",),
            vmem_limit_bytes=64 * 1024 * 1024,
        ),
    )(q3, k3, v3)
    return out.reshape(B, H, Sq, D)
```

```python
import functools
import math

import jax
import jax.numpy as jnp
import jax.experimental.pallas as pl
import jax.experimental.pallas.tpu as pltpu

_G = 4
_NB = 19
_P0 = 4
_E = 4
_W0 = 49
_WS = 2
_WROWS = 128


def _attn_kernel(q_hbm, k_hbm, v_hbm, o_hbm, qb, kb, vb, ob, qs, ks, vs, wsem,
                 *, c, B, H, Sq, Sk):
    G, NB, P0, E, W0, WS = _G, _NB, _P0, _E, _W0, _WS
    n = B * H // G
    gps = B // G

    def start_in(j, slot):
        h = j // gps
        b0 = (j % gps) * G
        for u in range(G):
            for hbm, buf, sem, S in ((k_hbm, kb, ks, Sk), (q_hbm, qb, qs, Sq),
                                     (v_hbm, vb, vs, Sk)):
                half = S // 2
                for t in range(2):
                    rows = pl.ds(t * half, half)
                    pltpu.make_async_copy(hbm.at[b0 + u, h, rows],
                                          buf.at[slot, u, rows],
                                          sem.at[slot]).start(priority=t)

    def wait_in(slot):
        for buf, sem in ((kb, ks), (qb, qs), (vb, vs)):
            pltpu.make_async_copy(buf.at[slot], buf.at[slot], sem.at[slot]).wait()

    def start_out(h):
        for t, r in enumerate(range(0, Sq, _WROWS)):
            rows = pl.ds(r, _WROWS)
            pltpu.make_async_copy(ob.at[h, :, rows], o_hbm.at[:, h, rows],
                                  wsem).start(priority=t % 2)

    n_in = 0
    while (W0 + n_in < n and (n_in + 1) * WS <= H
           and (n_in + 1) * WS * gps <= W0 + n_in):
        n_in += 1

    for d in range(P0):
        start_in(d, d)

    def body(i, carry):
        slot = i % NB
        wait_in(slot)
        j1 = P0 + i + i // E

        @pl.when(j1 < n)
        def _():
            start_in(j1, j1 % NB)

        @pl.when(jnp.logical_and(i % E == E - 1, j1 + 1 < n))
        def _():
            start_in(j1 + 1, (j1 + 1) % NB)

        @pl.when(jnp.logical_and(i >= W0, i - W0 < n_in))
        def _():
            for t in range(WS):
                start_out((i - W0) * WS + t)

        h = i // gps
        b0 = (i % gps) * G
        for u in range(G):
            q = qb[slot, u]
            k = kb[slot, u]
            v = vb[slot, u]
            s = jax.lax.dot_general(q, k, (((1,), (1,)), ((), ())),
                                    preferred_element_type=jnp.float32)
            m = jnp.max(s, axis=-1, keepdims=True)
            p = jnp.exp2((s - m) * c)
            l = jnp.sum(p, axis=-1, keepdims=True)
            o = jnp.dot(p.astype(jnp.bfloat16), v,
                        preferred_element_type=jnp.float32)
            r = pl.reciprocal(l, approx=True)
            ob[h, b0 + u] = (o * r).astype(ob.dtype)
        return carry

    jax.lax.fori_loop(0, n, body, 0)
    for h in range(n_in * WS, H):
        start_out(h)
    pltpu.make_async_copy(o_hbm, o_hbm, wsem).wait()


@jax.jit
def pallas_standalone__mha_softmax__near_ridge_kernel(q, k, v):
    B, H, Sq, D = q.shape
    Sk = k.shape[2]
    c = (D ** -0.5) * math.log2(math.e)
    n = B * H // _G
    for i in range(n):
        jmax = min(n - 1, _P0 + i + i // _E + (1 if i % _E == _E - 1 else 0))
        assert jmax - _NB < i
    return pl.pallas_call(
        functools.partial(_attn_kernel, c=c, B=B, H=H, Sq=Sq, Sk=Sk),
        in_specs=[pl.BlockSpec(memory_space=pl.ANY)] * 3,
        out_specs=pl.BlockSpec(memory_space=pl.ANY),
        out_shape=jax.ShapeDtypeStruct((B, H, Sq, D), q.dtype),
        scratch_shapes=[
            pltpu.VMEM((_NB, _G, Sq, D), q.dtype),
            pltpu.VMEM((_NB, _G, Sk, D), k.dtype),
            pltpu.VMEM((_NB, _G, Sk, D), v.dtype),
            pltpu.VMEM((H, B, Sq, D), q.dtype),
            pltpu.SemaphoreType.DMA((_NB,)),
            pltpu.SemaphoreType.DMA((_NB,)),
            pltpu.SemaphoreType.DMA((_NB,)),
            pltpu.SemaphoreType.DMA(()),
        ],
        compiler_params=pltpu.CompilerParams(
            vmem_limit_bytes=100 * 1024 * 1024,
            disable_bounds_checks=True,
        ),
    )(q, k, v)
```

```python
import functools
import math

import jax
import jax.numpy as jnp
import jax.experimental.pallas as pl
import jax.experimental.pallas.tpu as pltpu

_G = 4
_NB = 19
_P0 = 4
_E = 4
_W0 = 49
_WS = 3
_WROWS = 128


def _attn_kernel(q_hbm, k_hbm, v_hbm, o_hbm, qb, kb, vb, ob, qs, ks, vs, wsem,
                 *, c, B, H, Sq, Sk, G, NB, P0, E, W0, WS, WROWS):
    n = B * H // G
    gps = B // G

    def start_in(j, slot):
        h = j // gps
        b0 = (j % gps) * G
        for u in range(G):
            for hbm, buf, sem, S in ((k_hbm, kb, ks, Sk), (q_hbm, qb, qs, Sq),
                                     (v_hbm, vb, vs, Sk)):
                half = S // 2
                for t in range(2):
                    rows = pl.ds(t * half, half)
                    pltpu.make_async_copy(hbm.at[b0 + u, h, rows],
                                          buf.at[slot, u, rows],
                                          sem.at[slot]).start(priority=t)

    def wait_in(slot):
        for buf, sem in ((kb, ks), (qb, qs), (vb, vs)):
            pltpu.make_async_copy(buf.at[slot], buf.at[slot], sem.at[slot]).wait()

    def start_out(s):
        for r in range(0, Sq, WROWS):
            rows = pl.ds(r, WROWS)
            pltpu.make_async_copy(ob.at[s, :, rows], o_hbm.at[:, s, rows],
                                  wsem).start()

    def written(i):
        mn = min if isinstance(i, int) else jnp.minimum
        return mn(WS * (i - W0 + 1), i // gps)

    for d in range(P0):
        start_in(d, d)

    def body(i, carry):
        slot = i % NB
        wait_in(slot)
        j1 = P0 + i + i // E

        @pl.when(j1 < n)
        def _():
            start_in(j1, j1 % NB)

        @pl.when(jnp.logical_and(i % E == E - 1, j1 + 1 < n))
        def _():
            start_in(j1 + 1, (j1 + 1) % NB)

        @pl.when(i >= W0)
        def _():
            lo = jnp.where(i == W0, 0, written(i - 1))
            hi = written(i)
            for t in range(WS):
                @pl.when(lo + t < hi)
                def _():
                    start_out(lo + t)

        h = i // gps
        b0 = (i % gps) * G
        for u in range(G):
            q = qb[slot, u]
            k = kb[slot, u]
            v = vb[slot, u]
            s = jax.lax.dot_general(q, k, (((1,), (1,)), ((), ())),
                                    preferred_element_type=jnp.float32)
            m = jnp.max(s, axis=-1, keepdims=True)
            p = jnp.exp2((s - m) * c)
            l = jnp.sum(p, axis=-1, keepdims=True)
            o = jnp.dot(p.astype(v.dtype), v, preferred_element_type=jnp.float32)
            ob[h, b0 + u] = (o * pl.reciprocal(l, approx=True)).astype(ob.dtype)
        return carry

    jax.lax.fori_loop(0, n, body, 0)
    for s in range(written(n - 1), H):
        start_out(s)
    pltpu.make_async_copy(o_hbm, o_hbm, wsem).wait()


def _attention(q, k, v, *, G=_G, NB=_NB, P0=_P0, E=_E, W0=_W0, WS=_WS,
               WROWS=_WROWS, interpret=False):
    B, H, Sq, D = q.shape
    Sk = k.shape[2]
    n = B * H // G
    assert B % G == 0 and Sq % WROWS == 0 and P0 <= n and 1 <= W0 < n
    for i in range(n):
        jmax = min(n - 1, P0 + i + i // E + (1 if i % E == E - 1 else 0))
        assert jmax - NB < i
    c = (D ** -0.5) * math.log2(math.e)
    return pl.pallas_call(
        functools.partial(_attn_kernel, c=c, B=B, H=H, Sq=Sq, Sk=Sk, G=G, NB=NB,
                          P0=P0, E=E, W0=W0, WS=WS, WROWS=WROWS),
        in_specs=[pl.BlockSpec(memory_space=pl.ANY)] * 3,
        out_specs=pl.BlockSpec(memory_space=pl.ANY),
        out_shape=jax.ShapeDtypeStruct((B, H, Sq, D), q.dtype),
        scratch_shapes=[
            pltpu.VMEM((NB, G, Sq, D), q.dtype),
            pltpu.VMEM((NB, G, Sk, D), k.dtype),
            pltpu.VMEM((NB, G, Sk, D), v.dtype),
            pltpu.VMEM((H, B, Sq, D), q.dtype),
            pltpu.SemaphoreType.DMA((NB,)),
            pltpu.SemaphoreType.DMA((NB,)),
            pltpu.SemaphoreType.DMA((NB,)),
            pltpu.SemaphoreType.DMA(()),
        ],
        compiler_params=pltpu.CompilerParams(
            vmem_limit_bytes=96 * 1024 * 1024,
            disable_bounds_checks=True,
        ),
        interpret=interpret,
    )(q, k, v)


@jax.jit
def pallas_standalone__mha_softmax__near_ridge_kernel(q, k, v):
    return _attention(q, k, v)
```
